```python
import jax
import jax.numpy as jnp

def _softmax(x, axis=-1):
    return jax.nn.softmax(x, axis=axis)

def _gelu(x):
    return jax.nn.gelu(x, approximate=True)

def _silu(x):
    return jax.nn.silu(x)

def _sigmoid(x):
    return jax.nn.sigmoid(x)

def _layernorm(x, axis=-1, eps=1e-05):
    m = jnp.mean(x, axis=axis, keepdims=True)
    v = jnp.var(x, axis=axis, keepdims=True)
    return (x - m) / jnp.sqrt(v + eps)

def _scatter_add(tgt, idx, src, axis=0):
    return tgt.at[idx].add(src)

def _segment_sum(src, seg, n):
    return jax.ops.segment_sum(src, seg, n)

class _Rng:

    def __init__(self, key):
        self._k = key

    def _next(self):
        self._k, sub = jax.random.split(self._k)
        return sub

    def normal(self, shape):
        return jax.random.normal(self._next(), shape, dtype=jnp.bfloat16)

    def randint(self, lo, hi, shape):
        return jax.random.randint(self._next(), shape, lo, hi, dtype=jnp.int32)

    def uniform(self, shape, lo=0.0, hi=1.0):
        return jax.random.uniform(self._next(), shape, jnp.bfloat16, lo, hi)

    def permutation(self, n):
        return jax.random.permutation(self._next(), n)
kernel_name = 'adaLN_cond__sliding_block_cached__mixer_channel_mlp__decode'

def setup_inputs():
    _rng = _Rng(jax.random.key(int.from_bytes(__import__("os").urandom(4), "little")))
    _w = lambda a: (lambda t: t.astype(jnp.bfloat16) if jnp.issubdtype(t.dtype, jnp.floating) else t)(jnp.asarray(a))

    def _A_setup():
        B, Sq, D = (8, 1, 640)
        Hq, Hkv, Sk, Dh = (32, 32, 4096, 192)
        assert Hq % Hkv == 0, (Hq, Hkv)
        return {'x': _w((lambda *s: _rng.normal(s) * 0.05)(B, Sq, D)), 'k_cache': _w((lambda *s: _rng.normal(s) * 0.05)(B, Hkv, Sk, Dh)), 'v_cache': _w((lambda *s: _rng.normal(s) * 0.05)(B, Hkv, Sk, Dh)), 'wq': _w((lambda *s: _rng.normal(s) * 0.05)(D, Hq * Dh) * D ** (-0.5)), 'wo': _w((lambda *s: _rng.normal(s) * 0.05)(Hq * Dh, D) * (Hq * Dh) ** (-0.5))}
    _A_in = _A_setup()

    def _B_setup():
        B, S, D, F = (8, 1, 640, 1536)
        return {'x': _w((lambda *s: _rng.normal(s) * 0.05)(B, S, D)), 'w1': _w((lambda *s: _rng.normal(s) * 0.05)(D, F) * D ** (-0.5)), 'b1': _w((lambda *s: _rng.normal(s) * 0.05)(F)), 'w2': _w((lambda *s: _rng.normal(s) * 0.05)(F, D) * F ** (-0.5)), 'b2': _w((lambda *s: _rng.normal(s) * 0.05)(D))}
    _B_in = _B_setup()
    return {'A_x': _A_in['x'], 'A_k_cache': _A_in['k_cache'], 'A_v_cache': _A_in['v_cache'], 'A_wq': _A_in['wq'], 'A_wo': _A_in['wo'], 'B_x': _B_in['x'], 'B_w1': _B_in['w1'], 'B_b1': _B_in['b1'], 'B_w2': _B_in['w2'], 'B_b2': _B_in['b2'], 'c': _w((lambda *s: _rng.normal(s) * 0.05)(8, 640)), 'w_mod': _w((lambda *s: _rng.normal(s) * 0.05)(640, 6 * 640) * 640 ** (-0.5))}

def reference(A_x, A_k_cache, A_v_cache, A_wq, A_wo, B_x, B_w1, B_b1, B_w2, B_b2, c, w_mod):

    def _A_ref(x, k_cache, v_cache, wq, wo):
        B, Sq, D = x.shape
        Hq, Dh = (32, 192)
        Hkv, Sk = (k_cache.shape[1], k_cache.shape[2])
        W = min(4096, max(256, Sk // 4))
        rep = Hq // Hkv
        q = (lambda x, *d: x.transpose(*d))((x @ wq).reshape(B, Sq, Hq, Dh), 0, 2, 1, 3)
        k = jnp.repeat(k_cache[:, :, Sk - W:, :], rep, axis=1)
        v = jnp.repeat(v_cache[:, :, Sk - W:, :], rep, axis=1)
        scores = jnp.einsum('bhqd,bhkd->bhqk', q, k) * Dh ** (-0.5)
        p = _softmax(scores, axis=-1)
        o = jnp.einsum('bhqk,bhkd->bhqd', p, v)
        return (lambda x, *d: x.transpose(*d))(o, 0, 2, 1, 3).reshape(B, Sq, Hq * Dh) @ wo

    def _B_ref(x, w1, b1, w2, b2):
        y = _layernorm(x, axis=-1)
        h = _gelu(jnp.einsum('bsd,df->bsf', y, w1) + b1)
        return jnp.einsum('bsf,fd->bsd', h, w2) + b2
    x = A_x
    mod = (_silu(c) @ w_mod).reshape(c.shape[0], 6, 1, -1)
    sa, ca, ga, sb, cb, gb = (mod[:, 0].copy(), mod[:, 1].copy(), mod[:, 2].copy(), mod[:, 3].copy(), mod[:, 4].copy(), mod[:, 5].copy())
    h = _layernorm(x, axis=-1) * (1 + ca) + sa
    x = x + ga * _A_ref(h, A_k_cache, A_v_cache, A_wq, A_wo)
    h = _layernorm(x, axis=-1) * (1 + cb) + sb
    x = x + gb * _B_ref(h, B_w1, B_b1, B_w2, B_b2)
    return x
```

```python
import jax
import jax.numpy as jnp
from jax import lax
import jax.experimental.pallas as pl
import jax.experimental.pallas.tpu as pltpu

_HQ, _DH = 32, 192
_G = 8
_NBUF = 3
_EPS = 1e-5
_LANES = 128


def _layernorm(x):
    m = jnp.mean(x, axis=-1, keepdims=True)
    d = x - m
    v = jnp.mean(d * d, axis=-1, keepdims=True)
    return d / jnp.sqrt(v + _EPS)


def _dot(a, b):
    return jnp.dot(a.astype(jnp.bfloat16), b, preferred_element_type=jnp.float32)


def _row_bias(ref, rows):
    b = ref[...].astype(jnp.float32)
    return jnp.concatenate(
        [jnp.broadcast_to(b[t:t + 1, :], (rows, _LANES)) for t in range(b.shape[0])],
        axis=1,
    )


def _make_kernel(B, D, S, W):
    GD = _G * _DH
    NJ = _HQ // _G
    NCH = B * NJ
    scale = _DH ** -0.5

    def kernel(x_hbm, k_hbm, v_hbm, wq_hbm, wo_hbm, w1_hbm, b1_hbm, w2_hbm, b2_hbm,
               c_hbm, wmod_hbm, out_ref,
               x_v, c_v, b1_v, b2_v, wma_v, wmb_v, wq_v, wo_v, w1_v, w2_v,
               kbuf, vbuf, q_v, o_v, wsem, kvsem):
        def kv_copies(i, slot):
            rows = pl.ds(pl.multiple_of(i * GD, GD), GD)
            win = pl.ds(S - W, W)
            return (
                pltpu.make_async_copy(k_hbm.at[rows, win], kbuf.at[slot], kvsem.at[0, slot]),
                pltpu.make_async_copy(v_hbm.at[rows, win], vbuf.at[slot], kvsem.at[1, slot]),
            )

        cp_c = pltpu.make_async_copy(c_hbm, c_v, wsem.at[0])
        cp_x = pltpu.make_async_copy(x_hbm, x_v, wsem.at[1])
        cp_wma = pltpu.make_async_copy(wmod_hbm.at[:, pl.ds(0, 2 * D)], wma_v, wsem.at[2])
        cp_wq = pltpu.make_async_copy(wq_hbm, wq_v, wsem.at[3])
        cp_wmb = pltpu.make_async_copy(wmod_hbm.at[:, pl.ds(2 * D, 4 * D)], wmb_v, wsem.at[4])
        cp_wo = pltpu.make_async_copy(wo_hbm, wo_v, wsem.at[5])
        cp_b1 = pltpu.make_async_copy(b1_hbm, b1_v, wsem.at[6])
        cp_b2 = pltpu.make_async_copy(b2_hbm, b2_v, wsem.at[7])
        cp_w1 = pltpu.make_async_copy(w1_hbm, w1_v, wsem.at[8])
        cp_w2 = pltpu.make_async_copy(w2_hbm, w2_v, wsem.at[9])

        cp_wma.start()
        cp_c.start()
        cp_x.start()
        cp_wq.start()
        for i in range(_NBUF):
            for cp in kv_copies(i, i):
                cp.start()
        cp_b1.start()
        cp_b2.start()

        cp_c.wait()
        cp_x.wait()
        c = c_v[...].astype(jnp.float32)
        sc = (c * jax.nn.sigmoid(c)).astype(jnp.bfloat16)
        x = x_v[...].astype(jnp.float32)
        xn = _layernorm(x)
        cp_wma.wait()
        mod_a = _dot(sc, wma_v[...])
        h = (xn * (1.0 + mod_a[:, D:]) + mod_a[:, :D]).astype(jnp.bfloat16)
        cp_wq.wait()
        for j in range(NJ):
            q_v[j] = _dot(h, wq_v[:, j * GD:(j + 1) * GD])

        lane = lax.broadcasted_iota(jnp.int32, (_G, GD), 1)
        head = lax.broadcasted_iota(jnp.int32, (_G, GD), 0)
        diag = (lane >= head * _DH) & (lane < (head + 1) * _DH)

        def chunk(i, slot):
            b = i // NJ
            j = i % NJ
            cp_k, cp_v = kv_copies(i, slot)
            q = jnp.where(diag, q_v[j, pl.ds(b, 1), :], 0.0)
            cp_k.wait()
            s = _dot(q, kbuf[slot]) * scale
            e = jnp.exp(s - jnp.max(s, axis=-1, keepdims=True))
            p = (e / jnp.sum(e, axis=-1, keepdims=True)).astype(jnp.bfloat16)
            cp_v.wait()
            o = lax.dot_general(p, vbuf[slot], (((1,), (1,)), ((), ())),
                                preferred_element_type=jnp.float32)
            o_v[j, pl.ds(b, 1), :] = jnp.sum(jnp.where(diag, o, 0.0), axis=0, keepdims=True)

        def body(i, carry):
            slot = i % _NBUF
            chunk(i, slot)
            for cp in kv_copies(i + _NBUF, slot):
                cp.start()
            return carry

        lax.fori_loop(0, NCH - _NBUF, body, None)

        tail = [[cp_wmb, cp_wo], [cp_w1], [cp_w2]]
        for t in range(_NBUF):
            i = NCH - _NBUF + t
            chunk(i, i % _NBUF)
            for cp in tail[t] if t < len(tail) else []:
                cp.start()

        cp_wmb.wait()
        mod_b = _dot(sc, wmb_v[...])
        ga, sb, cb, gb = (mod_b[:, n * D:(n + 1) * D] for n in range(4))
        cp_wo.wait()
        attn = _dot(o_v[0], wo_v[0:GD, :])
        for j in range(1, NJ):
            attn += _dot(o_v[j], wo_v[j * GD:(j + 1) * GD, :])
        x1 = x + ga * attn
        y = _layernorm(_layernorm(x1) * (1.0 + cb) + sb)
        cp_b1.wait()
        cp_b2.wait()
        cp_w1.wait()
        hid = jax.nn.gelu(_dot(y, w1_v[...]) + _row_bias(b1_v, B), approximate=True)
        cp_w2.wait()
        mlp = _dot(hid, w2_v[...]) + _row_bias(b2_v, B)
        out_ref[...] = (x1 + gb * mlp).astype(out_ref.dtype)

    return kernel


@jax.jit
def pallas_adaLN_cond__sliding_block_cached__mixer_channel_mlp__decode_kernel(
    A_x: jax.Array,
    A_k_cache: jax.Array,
    A_v_cache: jax.Array,
    A_wq: jax.Array,
    A_wo: jax.Array,
    B_x: jax.Array,
    B_w1: jax.Array,
    B_b1: jax.Array,
    B_w2: jax.Array,
    B_b2: jax.Array,
    c: jax.Array,
    w_mod: jax.Array,
):
    del B_x
    B, Sq, D = A_x.shape
    _, Hkv, S, Dh = A_k_cache.shape
    F = B_w1.shape[1]
    assert Sq == 1 and Hkv == _HQ and Dh == _DH
    W = min(4096, max(256, S // 4))
    GD = _G * _DH
    bf16, f32 = jnp.bfloat16, jnp.float32

    kt = jnp.swapaxes(A_k_cache, 2, 3).reshape(B * Hkv * Dh, S)
    vt = jnp.swapaxes(A_v_cache, 2, 3).reshape(B * Hkv * Dh, S)

    out = pl.pallas_call(
        _make_kernel(B, D, S, W),
        out_shape=jax.ShapeDtypeStruct((B, D), A_x.dtype),
        in_specs=[pl.BlockSpec(memory_space=pl.ANY)] * 11,
        out_specs=pl.BlockSpec(memory_space=pltpu.VMEM),
        scratch_shapes=[
            pltpu.VMEM((B, D), bf16),
            pltpu.VMEM((B, D), bf16),
            pltpu.VMEM((F // _LANES, _LANES), bf16),
            pltpu.VMEM((D // _LANES, _LANES), bf16),
            pltpu.VMEM((D, 2 * D), bf16),
            pltpu.VMEM((D, 4 * D), bf16),
            pltpu.VMEM((D, _HQ * _DH), bf16),
            pltpu.VMEM((_HQ * _DH, D), bf16),
            pltpu.VMEM((D, F), bf16),
            pltpu.VMEM((F, D), bf16),
            pltpu.VMEM((_NBUF, GD, W), bf16),
            pltpu.VMEM((_NBUF, GD, W), bf16),
            pltpu.VMEM((_HQ // _G, B, GD), f32),
            pltpu.VMEM((_HQ // _G, B, GD), f32),
            pltpu.SemaphoreType.DMA((10,)),
            pltpu.SemaphoreType.DMA((2, _NBUF)),
        ],
        compiler_params=pltpu.CompilerParams(vmem_limit_bytes=100 * 1024 * 1024),
    )(
        A_x.reshape(B, D), kt, vt, A_wq, A_wo, B_w1,
        B_b1.reshape(F // _LANES, _LANES), B_w2, B_b2.reshape(D // _LANES, _LANES),
        c, w_mod,
    )
    return out.reshape(B, Sq, D)
```

```python
import jax
import jax.numpy as jnp
from jax import lax
import jax.experimental.pallas as pl
import jax.experimental.pallas.tpu as pltpu

_HQ, _DH = 32, 192
_EPS = 1e-5
_LANES = 128
_G = 8
_NBUF = 3
_KV_PIECE = 128
_W2_TAIL = (256, 128)


def _layernorm(x):
    m = jnp.mean(x, axis=-1, keepdims=True)
    d = x - m
    v = jnp.mean(d * d, axis=-1, keepdims=True)
    return d / jnp.sqrt(v + _EPS)


def _dot(a, b):
    return jnp.dot(a.astype(jnp.bfloat16), b, preferred_element_type=jnp.float32)


def _row_bias(ref, rows):
    b = ref[...].astype(jnp.float32)
    return jnp.concatenate(
        [jnp.broadcast_to(b[t:t + 1, :], (rows, _LANES)) for t in range(b.shape[0])],
        axis=1,
    )


def _make_kernel(B, D, F, S, W):
    GD = _G * _DH
    NJ = _HQ // _G
    NCH = B * NJ
    scale = _DH ** -0.5
    w2_len = (F - sum(_W2_TAIL),) + _W2_TAIL
    w2_off = tuple(sum(w2_len[:t]) for t in range(len(w2_len)))

    def kernel(x_hbm, k_hbm, v_hbm, wq_hbm, wo_hbm, w1_hbm, b1_hbm, w2_hbm, b2_hbm,
               c_hbm, wmod_hbm, out_ref,
               x_v, c_v, b1_v, b2_v, wmod_v, wq_v, wo_v, w1_v, w2_v,
               kv_v, q_v, o_v, mod_v):

        def stream(wsem, kvsem):
            def kv_start(i, slot):
                win = pl.ds(S - W, W)
                for r in range(0, GD, _KV_PIECE):
                    src = pl.ds(pl.multiple_of(i * GD + r, _KV_PIECE), _KV_PIECE)
                    for t, hbm in enumerate((k_hbm, v_hbm)):
                        pltpu.make_async_copy(
                            hbm.at[src, win],
                            kv_v.at[slot, t, pl.ds(r, _KV_PIECE)],
                            kvsem.at[slot],
                        ).start()

            def kv_wait(slot):
                pltpu.make_async_copy(kv_v.at[slot], kv_v.at[slot], kvsem.at[slot]).wait()

            small = [
                pltpu.make_async_copy(src, dst, wsem.at[0])
                for src, dst in ((c_hbm, c_v), (x_hbm, x_v), (b1_hbm, b1_v), (b2_hbm, b2_v))
            ]
            cp_wmod = pltpu.make_async_copy(wmod_hbm, wmod_v, wsem.at[1])
            cp_wq = pltpu.make_async_copy(wq_hbm, wq_v, wsem.at[2])
            cp_wo = pltpu.make_async_copy(wo_hbm, wo_v, wsem.at[0])
            cp_w1 = pltpu.make_async_copy(w1_hbm, w1_v, wsem.at[1])
            cp_w2 = [
                pltpu.make_async_copy(w2_hbm.at[pl.ds(o, n)], w2_v.at[pl.ds(o, n)], wsem.at[s])
                for o, n, s in zip(w2_off, w2_len, (2, 0, 1))
            ]

            cp_wmod.start()
            for cp in small:
                cp.start()
            cp_wq.start()
            lax.fori_loop(0, _NBUF, lambda i, _: kv_start(i, i), None)

            for cp in small:
                cp.wait()
            c = c_v[...].astype(jnp.float32)
            silu_c = (c * jax.nn.sigmoid(c)).astype(jnp.bfloat16)
            xn = _layernorm(x_v[...].astype(jnp.float32))
            cp_wmod.wait()
            mod_a = _dot(silu_c, wmod_v[:, :2 * D])
            h = (xn * (1.0 + mod_a[:, D:]) + mod_a[:, :D]).astype(jnp.bfloat16)
            mod_v[...] = _dot(silu_c, wmod_v[:, 2 * D:])
            cp_wq.wait()
            for j in range(NJ):
                q_v[j] = _dot(h, wq_v[:, j * GD:(j + 1) * GD])

            lane = lax.broadcasted_iota(jnp.int32, (_G, GD), 1)
            head = lax.broadcasted_iota(jnp.int32, (_G, GD), 0)
            diag = (lane >= head * _DH) & (lane < (head + 1) * _DH)

            def chunk(i, carry):
                slot = i % _NBUF
                b = i // NJ
                j = i % NJ
                kv_wait(slot)
                for t, cp in enumerate((cp_wo, cp_w1, cp_w2[0])):
                    pl.when(i == NCH - _NBUF + t)(cp.start)

                q = jnp.where(diag, q_v[j, pl.ds(b, 1), :], 0.0)
                s = _dot(q, kv_v[slot, 0]) * scale
                e = jnp.exp(s - jnp.max(s, axis=-1, keepdims=True))
                p = (e / jnp.sum(e, axis=-1, keepdims=True)).astype(jnp.bfloat16)
                o = lax.dot_general(p, kv_v[slot, 1], (((1,), (1,)), ((), ())),
                                    preferred_element_type=jnp.float32)
                o_v[j, pl.ds(b, 1), :] = jnp.sum(jnp.where(diag, o, 0.0), axis=0, keepdims=True)

                @pl.when(i + _NBUF < NCH)
                def _():
                    kv_start(i + _NBUF, slot)

                return carry

            lax.fori_loop(0, NCH, chunk, None)

            cp_wo.wait()
            cp_w2[1].start()
            ga, sb, cb, gb = (mod_v[:, n * D:(n + 1) * D] for n in range(4))
            attn = _dot(o_v[0], wo_v[0:GD, :])
            for j in range(1, NJ):
                attn += _dot(o_v[j], wo_v[j * GD:(j + 1) * GD, :])
            x1 = x_v[...].astype(jnp.float32) + ga * attn
            y = _layernorm(_layernorm(x1) * (1.0 + cb) + sb)
            cp_w1.wait()
            cp_w2[2].start()
            hid = jax.nn.gelu(_dot(y, w1_v[...]) + _row_bias(b1_v, B), approximate=True)
            hid = hid.astype(jnp.bfloat16)
            mlp = _row_bias(b2_v, B)
            for cp, o, n in zip(cp_w2, w2_off, w2_len):
                cp.wait()
                mlp += _dot(hid[:, o:o + n], w2_v[o:o + n, :])
            out_ref[...] = (x1 + gb * mlp).astype(out_ref.dtype)

        pl.run_scoped(
            stream, pltpu.SemaphoreType.DMA((3,)), pltpu.SemaphoreType.DMA((_NBUF,))
        )

    return kernel


@jax.jit
def pallas_adaLN_cond__sliding_block_cached__mixer_channel_mlp__decode_kernel(
    A_x: jax.Array,
    A_k_cache: jax.Array,
    A_v_cache: jax.Array,
    A_wq: jax.Array,
    A_wo: jax.Array,
    B_x: jax.Array,
    B_w1: jax.Array,
    B_b1: jax.Array,
    B_w2: jax.Array,
    B_b2: jax.Array,
    c: jax.Array,
    w_mod: jax.Array,
):
    del B_x
    B, Sq, D = A_x.shape
    _, Hkv, S, Dh = A_k_cache.shape
    F = B_w1.shape[1]
    assert Sq == 1 and Hkv == _HQ and Dh == _DH
    W = min(4096, max(256, S // 4))
    GD = _G * _DH
    bf16, f32 = jnp.bfloat16, jnp.float32

    kt = jnp.swapaxes(A_k_cache, 2, 3).reshape(B * Hkv * Dh, S)
    vt = jnp.swapaxes(A_v_cache, 2, 3).reshape(B * Hkv * Dh, S)

    out = pl.pallas_call(
        _make_kernel(B, D, F, S, W),
        out_shape=jax.ShapeDtypeStruct((B, D), A_x.dtype),
        in_specs=[pl.BlockSpec(memory_space=pl.ANY)] * 11,
        out_specs=pl.BlockSpec(memory_space=pltpu.VMEM),
        scratch_shapes=[
            pltpu.VMEM((B, D), bf16),
            pltpu.VMEM((B, D), bf16),
            pltpu.VMEM((F // _LANES, _LANES), bf16),
            pltpu.VMEM((D // _LANES, _LANES), bf16),
            pltpu.VMEM((D, 6 * D), bf16),
            pltpu.VMEM((D, _HQ * _DH), bf16),
            pltpu.VMEM((_HQ * _DH, D), bf16),
            pltpu.VMEM((D, F), bf16),
            pltpu.VMEM((F, D), bf16),
            pltpu.VMEM((_NBUF, 2, GD, W), bf16),
            pltpu.VMEM((_HQ // _G, B, GD), f32),
            pltpu.VMEM((_HQ // _G, B, GD), f32),
            pltpu.VMEM((B, 4 * D), f32),
        ],
        compiler_params=pltpu.CompilerParams(vmem_limit_bytes=64 * 1024 * 1024),
    )(
        A_x.reshape(B, D), kt, vt, A_wq, A_wo, B_w1,
        B_b1.reshape(F // _LANES, _LANES), B_w2, B_b2.reshape(D // _LANES, _LANES),
        c, w_mod,
    )
    return out.reshape(B, Sq, D)
```
